```python
import jax
import jax.numpy as jnp

def _softmax(x, axis=-1):
    return jax.nn.softmax(x, axis=axis)
def _gelu(x):
    return jax.nn.gelu(x, approximate=True)
def _silu(x):
    return jax.nn.silu(x)
def _sigmoid(x):
    return jax.nn.sigmoid(x)
def _layernorm(x, axis=-1, eps=1e-5):
    m = jnp.mean(x, axis=axis, keepdims=True)
    v = jnp.var(x, axis=axis, keepdims=True)
    return (x - m) / jnp.sqrt(v + eps)
def _scatter_add(tgt, idx, src, axis=0):
    return tgt.at[idx].add(src)
def _segment_sum(src, seg, n):
    return jax.ops.segment_sum(src, seg, n)
class _Rng:
    def __init__(self, key):
        self._k = key
    def _next(self):
        self._k, sub = jax.random.split(self._k)
        return sub
    def normal(self, shape):
        return jax.random.normal(self._next(), shape, dtype=jnp.bfloat16)
    def randint(self, lo, hi, shape):
        return jax.random.randint(self._next(), shape, lo, hi, dtype=jnp.int32)
    def uniform(self, shape, lo=0.0, hi=1.0):
        return jax.random.uniform(self._next(), shape, jnp.bfloat16, lo, hi)
    def permutation(self, n):
        return jax.random.permutation(self._next(), n)


kernel_name = 'standalone__detection_seg_fpn_lateral__vision'

def setup_inputs():
    _rng = _Rng(jax.random.key(int.from_bytes(__import__("os").urandom(4), "little")))
    _w = (lambda a: (lambda t: t.astype(jnp.bfloat16) if jnp.issubdtype(t.dtype, jnp.floating) else t)(jnp.asarray(a)))
    H = W = (384 // 2) * 2
    C = 384
    k = 1
    return {
        "c_fine": _w((lambda *s: _rng.normal(s) * 0.05)(1, H, W, C)),
        "p_coarse": _w((lambda *s: _rng.normal(s) * 0.05)(1, H // 2, W // 2, C)),
        "w_lat": _w((lambda *s: _rng.normal(s) * 0.05)(C, C)),
        "w_out": _w((lambda *s: _rng.normal(s) * 0.05)(k, k, C, C)),
    }

def reference(c_fine, p_coarse, w_lat, w_out):
    B, H, W, C = c_fine.shape
    k = 1
    lat = jnp.einsum("bhwc,cd->bhwd", c_fine, w_lat)
    up = jnp.repeat(jnp.repeat(p_coarse, 2, axis=1), 2, axis=2)
    m = lat + up
    pad = k // 2
    mp = jnp.pad(m, ((0, 0), (pad, pad), (pad, pad), (0, 0)))
    o = None
    for di in range(k):
        for dj in range(k):
            t = jnp.einsum("bhwc,cd->bhwd", mp[:, di:di + H, dj:dj + W, :], w_out[di, dj])
            o = t if o is None else o + t
    return o
```

```python
import jax
import jax.numpy as jnp
from jax import lax
from jax.experimental import pallas as pl
from jax.experimental.pallas import tpu as pltpu

G = 2
M = 16
B = 3
A = 10
P = 32


def _loop(lo, hi, f):
    def body(i, carry):
        f(i)
        return carry
    lax.fori_loop(lo, hi, body, 0)


@jax.jit
def pallas_standalone__detection_seg_fpn_lateral__vision_kernel(
    c_fine: jax.Array,
    p_coarse: jax.Array,
    w_lat: jax.Array,
    w_out: jax.Array,
):
    batch, H, W, C = c_fine.shape
    Wh = W // 2
    n_groups = H // (2 * G)
    n = n_groups // M
    n_strips = W // P
    RC = 2 * G * M
    assert batch == 1 and w_out.shape[:2] == (1, 1)
    assert n * RC == H and n >= 2 and n_strips * P == W and C % 128 == 0

    def kernel(c_hbm, p_hbm, wl_hbm, wo_hbm, o_hbm,
               c_buf, p_buf, o_buf, wl_ref, wo_ref, wf_ref, q_ref,
               c_sem, p_sem, o_sem, w_sem):
        def c_in(k, j):
            return pltpu.make_async_copy(
                c_hbm.at[0, pl.ds((k * M + j) * 2 * G, 2 * G)],
                c_buf.at[k % 2, pl.ds(j * 2 * G, 2 * G)], c_sem.at[k % 2, j])

        def p_in(k, j):
            return pltpu.make_async_copy(
                p_hbm.at[0, pl.ds((k * M + j) * G, G)],
                p_buf.at[k % 2, pl.ds(j * G, G)], p_sem.at[k % 2, j])

        def o_out(k, i, r0=0, nr=RC, sem_row=None):
            col = pl.ds(pl.multiple_of(i * P, P), P)
            return pltpu.make_async_copy(
                o_buf.at[k % 2, pl.ds(r0, nr), col],
                o_hbm.at[0, pl.ds(k * RC + r0, nr), col],
                o_sem.at[k % 2 if sem_row is None else sem_row, i])

        def start_read(k):
            def f(j):
                c_in(k, j).start()
                p_in(k, j).start()
            _loop(0, M, f)

        wl_in = pltpu.make_async_copy(wl_hbm, wl_ref, w_sem.at[0])
        wo_in = pltpu.make_async_copy(wo_hbm.at[0, 0], wo_ref, w_sem.at[1])
        wl_in.start()
        wo_in.start()
        start_read(0)
        start_read(1)
        wl_in.wait()
        wo_in.wait()
        wf_ref[...] = jnp.dot(wl_ref[...], wo_ref[...],
                              preferred_element_type=jnp.float32).astype(wf_ref.dtype)

        def step(g):
            k = g // M
            j = g - k * M
            s = k % 2

            @pl.when((k == 0) | (j < B))
            def _():
                c_in(k, j).wait()
                p_in(k, j).wait()

            @pl.when((k > 0) & (j == B))
            def _():
                _loop(B, M, lambda jj: c_in(k, jj).wait())
                _loop(B, M - 1, lambda jj: p_in(k, jj).wait())
                _loop(0, n_strips, lambda i: o_out(k - 1, i).start())
                p_in(k, M - 1).wait()

            @pl.when((k > 0) & (j == A))
            def _():
                @pl.when(k + 1 < n)
                def _():
                    _loop(0, n_strips - 1, lambda i: o_out(k - 1, i).wait())
                    start_read(k + 1)
                    _loop(n_strips - 1, n_strips, lambda i: o_out(k - 1, i).wait())

                @pl.when(k + 1 == n)
                def _():
                    _loop(0, n_strips, lambda i: o_out(n - 1, i, 0, 2 * G * A).start())

            for r in range(G):
                u = j * G + r
                q = jnp.dot(p_buf[s, u], wo_ref[...], preferred_element_type=jnp.float32)
                for b in range(C // 128):
                    qb = q[:, b * 128:(b + 1) * 128]
                    q_ref[b, pl.ds(0, Wh, stride=2), :] = qb
                    q_ref[b, pl.ds(1, Wh, stride=2), :] = qb
                q_up = jnp.concatenate([q_ref[b] for b in range(C // 128)], axis=1)
                for i in range(2):
                    lat = jnp.dot(c_buf[s, 2 * u + i], wf_ref[...],
                                  preferred_element_type=jnp.float32)
                    o_buf[s, 2 * u + i] = (lat + q_up).astype(o_buf.dtype)

        _loop(0, n_groups, step)

        r0 = 2 * G * A
        _loop(0, n_strips, lambda i: o_out(n - 1, i, r0, RC - r0, 2).start())
        _loop(0, n_strips, lambda i: o_out(n - 2, i).wait())
        _loop(0, n_strips, lambda i: o_out(n - 1, i, 0, r0).wait())
        _loop(0, n_strips, lambda i: o_out(n - 1, i, r0, RC - r0, 2).wait())

    any_spec = pl.BlockSpec(memory_space=pl.ANY)
    dt = c_fine.dtype
    return pl.pallas_call(
        kernel,
        in_specs=[any_spec] * 4,
        out_specs=any_spec,
        out_shape=jax.ShapeDtypeStruct(c_fine.shape, dt),
        scratch_shapes=[
            pltpu.VMEM((2, RC, W, C), dt),
            pltpu.VMEM((2, RC // 2, Wh, C), dt),
            pltpu.VMEM((2, RC, W, C), dt),
            pltpu.VMEM((C, C), w_lat.dtype),
            pltpu.VMEM((C, C), w_out.dtype),
            pltpu.VMEM((C, C), dt),
            pltpu.VMEM((C // 128, W, 128), jnp.float32),
            pltpu.SemaphoreType.DMA((2, M)),
            pltpu.SemaphoreType.DMA((2, M)),
            pltpu.SemaphoreType.DMA((3, n_strips)),
            pltpu.SemaphoreType.DMA((2,)),
        ],
        compiler_params=pltpu.CompilerParams(vmem_limit_bytes=110 * 2**20),
    )(c_fine, p_coarse, w_lat, w_out)
```

```python
import jax
import jax.numpy as jnp
from jax import lax
from jax.experimental import pallas as pl
from jax.experimental.pallas import tpu as pltpu

G = 3
T = 2 * G
Q = 2
RING = 14
SWITCH = 38
BLOCK = 8
STRIP = 48
SWEEPS0 = 4


def _loop(lo, hi, f):
    def body(i, carry):
        f(i)
        return carry
    lax.fori_loop(lo, hi, body, 0)


@jax.jit
def pallas_standalone__detection_seg_fpn_lateral__vision_kernel(
    c_fine: jax.Array,
    p_coarse: jax.Array,
    w_lat: jax.Array,
    w_out: jax.Array,
):
    batch, H, W, C = c_fine.shape
    Wh = W // 2
    n_steps = H // T
    n_batches = n_steps // Q
    last = n_batches - 1
    assert batch == 1 and w_out.shape == (1, 1, C, C)
    assert n_batches * Q * T == H and n_steps % BLOCK == 0
    assert W % STRIP == 0 and C % 128 == 0
    assert 0 < (n_batches - RING) * Q <= SWITCH <= last * Q

    def kernel(c_hbm, p_hbm, wl_hbm, wo_hbm, o_hbm,
               buf, p_ring, wl_ref, wo_ref, wf_ref, q_ref, read_sems, sems):
        write_sem, aux_sem = sems.at[0], sems.at[1]

        def c_in(b):
            rows = pl.ds(b * Q, Q)
            return pltpu.make_async_copy(
                c_hbm.at[rows], buf.at[rows], read_sems.at[lax.rem(b, RING)])

        def p_in(b):
            slot = lax.rem(b, RING)
            return pltpu.make_async_copy(
                p_hbm.at[pl.ds(b * Q, Q)], p_ring.at[slot], read_sems.at[slot])

        def p_in_last():
            return pltpu.make_async_copy(
                p_hbm.at[pl.ds(last * Q, Q)], p_ring.at[last % RING], aux_sem)

        def start_batch(b):
            c_in(b).start()
            p_in(b).start()

        def wait_batch(b):
            c_in(b).wait()
            p_in(b).wait()

        def start_sweep(v):
            block = lax.div(v, T)
            for i in range(W // STRIP):
                idx = (pl.ds(block * BLOCK, BLOCK), v - block * T, pl.ds(i * STRIP, STRIP))
                pltpu.make_async_copy(buf.at[idx], o_hbm.at[idx], write_sem).start()

        def sweeps_started(g):
            paced = SWEEPS0 + lax.div(3 * (g - SWITCH), 2)
            return jnp.where(g < SWITCH, 0, jnp.minimum(paced, T * lax.div(g, BLOCK)))

        wl_in = pltpu.make_async_copy(wl_hbm, wl_ref, aux_sem)
        wo_in = pltpu.make_async_copy(wo_hbm, wo_ref, aux_sem)
        wl_in.start()
        wo_in.start()
        _loop(0, RING, start_batch)
        wl_in.wait()
        wo_in.wait()
        wf_ref[...] = jnp.dot(wl_ref[...], wo_ref[...],
                              preferred_element_type=jnp.float32).astype(wf_ref.dtype)

        def step(g):
            b = lax.div(g, Q)
            first = g == b * Q

            @pl.when(first & (b >= 1) & (b - 1 + RING < last))
            def _():
                start_batch(b - 1 + RING)

            @pl.when(g == (n_batches - RING) * Q)
            def _():
                _loop(last, n_batches, lambda bb: c_in(bb).start())
                p_in_last().start()

            @pl.when(first & (g < SWITCH))
            def _():
                wait_batch(b)

            @pl.when(g == SWITCH)
            def _():
                _loop(pl.cdiv(SWITCH, Q), last, wait_batch)
                c_in(last).wait()

            _loop(sweeps_started(g - 1), sweeps_started(g), start_sweep)

            @pl.when(g == SWITCH)
            def _():
                p_in_last().wait()

            for r in range(G):
                q = jnp.dot(p_ring[lax.rem(b, RING), g - b * Q, r], wo_ref[...],
                            preferred_element_type=jnp.float32)
                for l in range(C // 128):
                    q_l = q[:, l * 128:(l + 1) * 128]
                    q_ref[l, pl.ds(0, Wh, stride=2), :] = q_l
                    q_ref[l, pl.ds(1, Wh, stride=2), :] = q_l
                q_up = jnp.concatenate([q_ref[l] for l in range(C // 128)], axis=1)
                for i in (2 * r, 2 * r + 1):
                    lat = jnp.dot(buf[g, i], wf_ref[...],
                                  preferred_element_type=jnp.float32)
                    buf[g, i] = (lat + q_up).astype(buf.dtype)

        _loop(0, n_steps, step)

        _loop(sweeps_started(n_steps - 1), T * (n_steps // BLOCK), start_sweep)
        pltpu.make_async_copy(buf, o_hbm, write_sem).wait()

    any_spec = pl.BlockSpec(memory_space=pl.ANY)
    out = pl.pallas_call(
        kernel,
        in_specs=[any_spec] * 4,
        out_specs=any_spec,
        out_shape=jax.ShapeDtypeStruct((n_steps, T, W, C), c_fine.dtype),
        scratch_shapes=[
            pltpu.VMEM((n_steps, T, W, C), c_fine.dtype),
            pltpu.VMEM((RING, Q, G, Wh, C), p_coarse.dtype),
            pltpu.VMEM((C, C), w_lat.dtype),
            pltpu.VMEM((C, C), w_out.dtype),
            pltpu.VMEM((C, C), c_fine.dtype),
            pltpu.VMEM((C // 128, W, 128), jnp.float32),
            pltpu.SemaphoreType.DMA((RING,)),
            pltpu.SemaphoreType.DMA((2,)),
        ],
        compiler_params=pltpu.CompilerParams(vmem_limit_bytes=124 * 2**20),
    )(
        c_fine.reshape(n_steps, T, W, C),
        p_coarse.reshape(n_steps, G, Wh, C),
        w_lat,
        w_out.reshape(C, C),
    )
    return out.reshape(c_fine.shape)
```
